```python
import jax
import jax.numpy as jnp

def _softmax(x, axis=-1):
    return jax.nn.softmax(x, axis=axis)
def _gelu(x):
    return jax.nn.gelu(x, approximate=True)
def _silu(x):
    return jax.nn.silu(x)
def _sigmoid(x):
    return jax.nn.sigmoid(x)
def _layernorm(x, axis=-1, eps=1e-5):
    m = jnp.mean(x, axis=axis, keepdims=True)
    v = jnp.var(x, axis=axis, keepdims=True)
    return (x - m) / jnp.sqrt(v + eps)
def _scatter_add(tgt, idx, src, axis=0):
    return tgt.at[idx].add(src)
def _segment_sum(src, seg, n):
    return jax.ops.segment_sum(src, seg, n)
class _Rng:
    def __init__(self, key):
        self._k = key
    def _next(self):
        self._k, sub = jax.random.split(self._k)
        return sub
    def normal(self, shape):
        return jax.random.normal(self._next(), shape, dtype=jnp.bfloat16)
    def randint(self, lo, hi, shape):
        return jax.random.randint(self._next(), shape, lo, hi, dtype=jnp.int32)
    def uniform(self, shape, lo=0.0, hi=1.0):
        return jax.random.uniform(self._next(), shape, jnp.bfloat16, lo, hi)
    def permutation(self, n):
        return jax.random.permutation(self._next(), n)


kernel_name = 'standalone__modern_conv_block_convnext__vision'

def setup_inputs():
    _rng = _Rng(jax.random.key(int.from_bytes(__import__("os").urandom(4), "little")))
    _w = (lambda a: (lambda t: t.astype(jnp.bfloat16) if jnp.issubdtype(t.dtype, jnp.floating) else t)(jnp.asarray(a)))
    H = W = 512
    C = 96
    K = 3
    return {
        "x": _w((lambda *s: _rng.normal(s) * 0.05)(1, H, W, C)),
        "dw": _w((lambda *s: _rng.normal(s) * 0.05)(K, K, C)),
        "w1": _w((lambda *s: _rng.normal(s) * 0.05)(C, 4 * C)),
        "b1": _w((lambda *s: _rng.normal(s) * 0.05)(4 * C)),
        "w2": _w((lambda *s: _rng.normal(s) * 0.05)(4 * C, C)),
        "b2": _w((lambda *s: _rng.normal(s) * 0.05)(C)),
        "gamma": _w((lambda *s: _rng.normal(s) * 0.05)(C)),
    }

def reference(x, dw, w1, b1, w2, b2, gamma):
    B, H, W, C = x.shape
    K = dw.shape[0]
    pad = K // 2
    xp = jnp.pad(x, ((0,0),(pad,pad),(pad,pad),(0,0)))
    out = jnp.zeros_like(x)
    for i in range(K):
        for j in range(K):
            out = out + xp[:, i:i+H, j:j+W, :] * dw[i, j][None, None, None, :]
    h = _layernorm(out, axis=-1)
    h = jnp.einsum('bhwc,ce->bhwe', h, w1) + b1
    h = _gelu(h)
    h = jnp.einsum('bhwe,ec->bhwc', h, w2) + b2
    return x + gamma[None, None, None, :] * h
```

```python
import functools
import numpy as np
import jax
import jax.numpy as jnp
from jax import lax
from jax.experimental import pallas as pl
from jax.experimental.pallas import tpu as pltpu

def env(k, d):
    return d
TH = env('TH', 16)
OPQ = env('OPQ', 'hropy')
NHOP = env('NHOP', 0); PMEM = env('PMEM', 2); HMEM = env('HMEM', 1)
KPAD = env('KPAD', 1); STAT = env('STAT', 0); GM = env('GM', 0)
DIST = env('DIST', '0002')
PACK = env('PACK', 0); YV = env('YV', 0); AV = env('AV', 1)
FLAGS = {}
H = 512; W = 512; C = 96; E = 384
f32 = jnp.float32; bf16 = jnp.bfloat16; u32 = jnp.uint32
C1 = float(np.sqrt(2.0 / np.pi)); C2 = 0.044715
S = float((C1 * C2) ** (1.0 / 3.0)); KK = C1 / S
SHI = float(np.float32(S).astype(jnp.bfloat16).astype(np.float32)); SLO = float(np.float32(S) - np.float32(SHI))
NZ = 1024
NS = env('NS', 6); NXA = env('NXA', 3); NY = env('NY', 2); NH = 2; NP = 2
TAPS = [0, 1, 2, 3, 5, 6, 7, 8]

def kern(zz, xm_ref, xp_ref, xn_ref, dw_ref, w1_ref, b1_ref, w2t_ref, b2_ref, gam_ref, o_ref, *scr):
    k = 0
    def take(n):
        nonlocal k
        r = scr[k:k + n]; k += n
        return r
    xf = take(NS); xas = take(NXA); ybs = take(NY); hsc = take(NH); pms = take(NP)
    w1s, w2s, gbs, dsc, dwb_ref = take(5)
    xps = take(NS)
    i = pl.program_id(0)
    nb = pl.num_programs(0)
    zc = [0]
    def Z(kind):
        if kind in OPQ:
            zc[0] += 1
            return zz[zc[0] % NZ]
        return 0

    @pl.when(i == 0)
    def _():
        def col(rowv):
            r = jnp.concatenate([rowv, jnp.zeros((1, 128 - C), f32)], axis=1)
            return jnp.broadcast_to(r, (128, 128)).T[:C]
        dwv = dw_ref[...].astype(f32)
        for ii in range(3):
            for jj in range(3):
                dwb_ref[0, ii * 3 + jj] = col(dwv[ii, jj:jj + 1, :])
        gam = gam_ref[...].astype(f32).reshape(1, C)
        b2v = b2_ref[...].astype(f32).reshape(1, C)
        gbs[0] = col(gam * b2v)
        gsc_ = col(gam * (0.5 / S))
        for kk in range(3):
            w2s[0, kk] = pltpu.bitcast((w2t_ref[:, kk * 128:(kk + 1) * 128].astype(f32) * gsc_).astype(bf16), u32)
        w1f = w1_ref[...].astype(f32)
        b1v = b1_ref[...].astype(f32).reshape(1, E)
        cs = -jnp.sum(w1f, axis=0, keepdims=True)
        s8 = lax.broadcasted_iota(jnp.int32, (8, E), 0)
        ex = jnp.where(s8 < 2, b1v, jnp.where(s8 == 2, cs if KPAD else 0.0, 0.0))
        w1p = jnp.concatenate([w1f, ex, jnp.zeros((24, E), f32)], axis=0)
        w1s[0] = pltpu.bitcast(w1p.T.astype(bf16), u32)
        sub = lax.broadcasted_iota(jnp.int32, (32, W), 0)
        padc = jnp.where(sub == 0, SHI, jnp.where(sub == 1, SLO, 0.0)).astype(f32)
        for xa in xas: xa[0, C:, :] = padc
        r16 = lax.broadcasted_iota(jnp.int32, (16, 128), 0); l16 = lax.broadcasted_iota(jnp.int32, (16, 128), 1)
        for q in range(GM):
            d = jnp.zeros((16, 128), f32)
            for ti, tap in enumerate(TAPS):
                d = jnp.where(l16 == r16 + 16 * ti, dwb_ref[0, tap, 16 * q:16 * q + 16, :], d)
            dsc[0, q] = pltpu.bitcast(d.astype(bf16), u32)

    lane = lax.broadcasted_iota(jnp.int32, (8, 128), 1)
    sub8 = lax.broadcasted_iota(jnp.int32, (8, 128), 0)
    m_first = lane == 0
    m_last = lane == 127

    def unpack(v):
        s = (v + 1) % NS
        ok = None
        if v < 0: src = xp_ref.at[0]; ok = i > 0
        elif v >= TH: src = xn_ref.at[0]; ok = i < nb - 1
        else: src = xm_ref.at[v]
        x = src[...].astype(f32)
        if ok is not None: x = jnp.where(ok, x, 0.0)
        xf[s][0] = x
        if GM:
            pk = pltpu.bitcast(src[0:16 * GM, :], u32)
            if ok is not None: pk = jnp.where(ok, pk, jnp.zeros((), u32))
            xps[s][0, 0] = pk
            z0 = jnp.zeros((8, 128), u32)
            for q in range(GM):
                sl = slice(8 * q, 8 * q + 8)
                pm = [pltpu.roll(pk[sl, t * 128:(t + 1) * 128], 1, 1) for t in range(4)]
                pp = [pltpu.roll(pk[sl, t * 128:(t + 1) * 128], 127, 1) for t in range(4)]
                for t in range(4):
                    ln = slice(t * 128, (t + 1) * 128)
                    xps[s][0, 1, sl, ln] = jnp.where(m_first, pm[t - 1] if t > 0 else z0, pm[t])
                    xps[s][0, 2, sl, ln] = jnp.where(m_last, pp[t + 1] if t < 3 else z0, pp[t])
    XF = lambda v: xf[(v + 1) % NS]
    XP = lambda v: xps[(v + 1) % NS]

    AS = {}
    def acc(v, t, y, sl, ln):
        st = AS[v]
        if YV: st.setdefault('y', {})[(sl.start, ln.start)] = y
        else: ybs[v % NY][0, sl, ln] = y
        st['s1'][t] = y if st['s1'][t] is None else st['s1'][t] + y
        st['s2'][t] = y * y if st['s2'][t] is None else st['s2'][t] + y * y
    def a_begin(v):
        AS[v] = dict(s1=[None] * 4, s2=[None] * 4, za=[Z('x') for _ in range(3)], zd=Z('d'), zp=[Z('q') for _ in range(3)])
    def a_mxu(v, q):
        st = AS[v]
        parts = []
        for tap in TAPS:
            ii, j = divmod(tap, 3)
            parts.append(pltpu.bitcast(XP(v - 1 + ii)[st['zp'][ii], (1, 0, 2)[j], 8 * q:8 * q + 8, :], bf16))
        rhs = jnp.concatenate(parts, axis=0)
        y = jnp.dot(pltpu.bitcast(dsc[st['zd'], q], bf16), rhs, preferred_element_type=f32)
        for hh in range(2):
            sl = slice(16 * q + 8 * hh, 16 * q + 8 * hh + 8)
            w4 = dwb_ref[st['zd'], 4, sl, :]
            for t in range(4):
                ln = slice(t * 128, (t + 1) * 128)
                acc(v, t, y[8 * hh:8 * hh + 8, ln] + XF(v)[st['za'][1], sl, ln] * w4, sl, ln)
    def a_valu(v, g):
        st = AS[v]; za = st['za']
        sl = slice(g * 8, (g + 1) * 8)
        wts = [dwb_ref[st['zd'], kk, sl, :] for kk in range(9)]
        ym = []; y0 = []; yp = []
        for t in range(4):
            ln = slice(t * 128, (t + 1) * 128)
            a = XF(v - 1)[za[0], sl, ln]; b = XF(v)[za[1], sl, ln]; c = XF(v + 1)[za[2], sl, ln]
            ym.append(pltpu.roll(a * wts[0] + b * wts[3] + c * wts[6], 1, 1))
            y0.append(a * wts[1] + b * wts[4] + c * wts[7])
            yp.append(pltpu.roll(a * wts[2] + b * wts[5] + c * wts[8], 127, 1))
        for t in range(4):
            ln = slice(t * 128, (t + 1) * 128)
            l = jnp.where(m_first, ym[t - 1] if t > 0 else 0.0, ym[t])
            rr = jnp.where(m_last, yp[t + 1] if t < 3 else 0.0, yp[t])
            acc(v, t, y0[t] + l + rr, sl, ln)
    def a_ln(v):
        st = AS.pop(v); s1 = st['s1']; s2 = st['s2']
        yb = ybs[v % NY]; xa = xas[v % NXA]
        zy = Z('y')
        pc = jnp.where(sub8 == 0, SHI, jnp.where(sub8 == 1, SLO, 0.0)).astype(f32)
        def stats(a1, a2):
            m = a1 * (1.0 / C)
            vv = a2 * (1.0 / C) - m * m
            rs = lax.rsqrt(jnp.maximum(vv, 0.0) + 1e-5) * S
            return m, rs
        if STAT == 0:
            ms = []; rss = []
            for t in range(4):
                m, rs = stats(jnp.sum(s1[t], axis=0, keepdims=True), jnp.sum(s2[t], axis=0, keepdims=True))
                ms.append(jnp.broadcast_to(m, (8, 128))); rss.append(jnp.broadcast_to(rs, (8, 128)))
        else:
            def merge(vs):
                lo = sub8 < 4
                ev = (sub8 % 2) == 0
                def fold4(a): return a + pltpu.roll(a, 4, 0)
                def comb(a, b, sh, msk):
                    u = jnp.where(msk, a, b); w = jnp.where(msk, b, a)
                    return u + pltpu.roll(w, sh, 0) if False else u + rollx(w, sh, msk)
                def rollx(w, sh, msk):
                    return jnp.where(msk, pltpu.roll(w, 8 - sh, 0), pltpu.roll(w, sh, 0)) if sh != 4 else pltpu.roll(w, 4, 0)
                return None
            r1 = [jnp.broadcast_to(jnp.sum(s1[t], axis=0, keepdims=True), (8, 128)) for t in range(4)]
            r2 = [jnp.broadcast_to(jnp.sum(s2[t], axis=0, keepdims=True), (8, 128)) for t in range(4)]
            g1 = jnp.where(sub8 < 2, r1[0], jnp.where(sub8 < 4, r1[1], jnp.where(sub8 < 6, r1[2], r1[3])))
            g2 = jnp.where(sub8 < 2, r2[0], jnp.where(sub8 < 4, r2[1], jnp.where(sub8 < 6, r2[2], r2[3])))
            m, rs = stats(g1, g2)
            ms = [jnp.broadcast_to(m[2 * t:2 * t + 1, :], (8, 128)) for t in range(4)]
            rss = [jnp.broadcast_to(rs[2 * t:2 * t + 1, :], (8, 128)) for t in range(4)]
        cols = []
        for t in range(4):
            ln = slice(t * 128, (t + 1) * 128)
            rsb = rss[t]; mb = ms[t]
            for _ in range(NHOP): rsb = pltpu.roll(rsb, Z('r'), 1)
            parts = []
            for g in range(C // 8):
                sl = slice(g * 8, (g + 1) * 8)
                yy = st['y'][(sl.start, ln.start)] if YV else yb[zy, sl, ln]
                val = yy * rsb if KPAD else (yy - mb) * rsb
                if AV: parts.append(val)
                else: xa[0, sl, ln] = val
            pv = jnp.where(sub8 == 2, mb * rsb, pc) if KPAD else pc
            if AV:
                cols.append(jnp.concatenate(parts + [pv, jnp.zeros((24, 128), f32)], axis=0))
            elif KPAD:
                xa[0, 96:104, ln] = pv
        if AV: XAV[v] = jnp.concatenate(cols, axis=1)
    XAV = {}

    def mm1(v):
        w1 = pltpu.bitcast(w1s[Z('w')], bf16)
        hsc[v % NH][0] = jnp.dot(w1, XAV.pop(v) if AV else xas[v % NXA][Z('a')], preferred_element_type=f32)
    def mm2(v, hook):
        zw = Z('w')
        h = hsc[v % NH][Z('h')]
        g = h + h * jnp.tanh(h * (h * h + KK))
        gb = jnp.concatenate([gbs[zw]] * 4, axis=1)
        pm = pms[v % NP]
        npm = 3 if PMEM == 1 else 2
        last = None
        for kk in range(3):
            p = jnp.dot(pltpu.bitcast(w2s[zw, kk], bf16), g[kk * 128:(kk + 1) * 128], preferred_element_type=f32)
            if kk < npm: pm[0, kk] = p
            else: last = p
            hook(kk + 1)
        zp = Z('p')
        a = pm[zp, 0] + pm[zp, 1]
        a = a + (pm[zp, 2] if PMEM == 1 else last)
        o_ref[v] = (a + (XF(v)[Z('o')] + gb)).astype(bf16)

    def stageA_parts(v):
        unpack(v + 1); a_begin(v)
        return [functools.partial(a_mxu, v, q) for q in range(GM)], [functools.partial(a_valu, v, g) for g in range(2 * GM, C // 8)]
    unpack(-1); unpack(0)
    AL = env('AL', 1)
    for v in range(AL):
        mx, va = stageA_parts(v)
        for o in mx + va: o()
        a_ln(v)
    nxt = AL
    if AL == 1 or True:
        pass
    mm1(0)
    D = [int(c) for c in DIST]
    for r in range(TH):
        m = r + AL
        mx, va = ([], [])
        if m < TH: mx, va = stageA_parts(m)
        q = [0]
        def hook(hh):
            for _ in range(D[hh]):
                if q[0] < len(mx): mx[q[0]](); q[0] += 1
        if AL == 1 or not GM:
            for o in mx + va: o()
            q[0] = len(mx)
            if m < TH: a_ln(m)
            if r + 1 < TH: mm1(r + 1)
            mm2(r, lambda hh: None)
        else:
            if r + 1 < TH: mm1(r + 1)
            hook(0)
            mm2(r, hook)
            while q[0] < len(mx): mx[q[0]](); q[0] += 1
            for o in va: o()
            if m < TH: a_ln(m)

@jax.jit
def pallas_standalone__modern_conv_block_convnext__vision_kernel(x, dw, w1, b1, w2, b2, gamma):
    xt = jnp.transpose(x[0], (0, 2, 1))
    w2t = w2.T
    nb = H // TH
    ND = env('NODMA', 0)
    zz = jnp.zeros((NZ,), jnp.int32)
    full = lambda a: pl.BlockSpec(a.shape, lambda i, z: (0,) * a.ndim)
    scr = [pltpu.VMEM((1, C, W), f32)] * NS + [pltpu.VMEM((1, 128, W), f32)] * NXA + [pltpu.VMEM((1, C, W), f32)] * NY
    scr += [pltpu.VMEM((1, E, W), f32)] * NH + [pltpu.VMEM((1, 3, C, W), f32)] * NP
    scr += [pltpu.VMEM((1, E // 2, 128), u32), pltpu.VMEM((1, 3, C // 2, 128), u32), pltpu.VMEM((1, C, 128), f32), pltpu.VMEM((1, max(GM, 1), 8, 128), u32), pltpu.VMEM((1, 9, C, 128), f32)]
    scr += [pltpu.VMEM((1, 3, 8 * max(GM, 1), W), u32)] * NS
    out = pl.pallas_call(
        kern,
        grid_spec=pltpu.PrefetchScalarGridSpec(
            num_scalar_prefetch=1, grid=(nb,),
            in_specs=[pl.BlockSpec((TH, C, W), lambda i, z: (i * (1 - ND), 0, 0)),
                  pl.BlockSpec((1, C, W), lambda i, z: (jnp.maximum(i * TH - 1, 0) * (1 - ND), 0, 0)),
                  pl.BlockSpec((1, C, W), lambda i, z: (jnp.minimum(i * TH + TH, H - 1) * (1 - ND), 0, 0)),
                  full(dw), full(w1), full(b1), full(w2t), full(b2), full(gamma)],
            out_specs=pl.BlockSpec((TH, C, W), lambda i, z: (i * (1 - ND), 0, 0)),
            scratch_shapes=scr),
        out_shape=jax.ShapeDtypeStruct((H, C, W), bf16),
        compiler_params=pltpu.CompilerParams(dimension_semantics=("arbitrary",), vmem_limit_bytes=110 * 1024 * 1024, flags=FLAGS),
    )(zz, xt, xt, xt, dw, w1, b1, w2t, b2, gamma)
    return jnp.transpose(out, (0, 2, 1))[None]
```

```python
import functools
import numpy as np
import jax
import jax.numpy as jnp
from jax import lax
from jax.experimental import pallas as pl
from jax.experimental.pallas import tpu as pltpu

def env(k, d):
    return d
TH = env('TH', 32); CH = env('CH', 16)
OPQ = env('OPQ', 'hropy')
NHOP = env('NHOP', 0); PMEM = env('PMEM', 2); GEL = env('GEL', 0); SACC = env('SACC', 1); OUTA = env('OUTA', 3); YA = env('YA', 1); HMEM = env('HMEM', 1); NOWAIT = env('NOWAIT', 1); LAGC = env('LAGC', 0)
KPAD = env('KPAD', 1); STAT = env('STAT', 0); GM = env('GM', 0)
DIST = env('DIST', '0002')
PACK = env('PACK', 0); YV = env('YV', 0); AV = env('AV', 1)
FLAGS = {}
H = 512; W = 512; C = 96; E = 384
f32 = jnp.float32; bf16 = jnp.bfloat16; u32 = jnp.uint32
C1 = float(np.sqrt(2.0 / np.pi)); C2 = 0.044715
S = float((C1 * C2) ** (1.0 / 3.0)); KK = C1 / S
SHI = float(np.float32(S).astype(jnp.bfloat16).astype(np.float32)); SLO = float(np.float32(S) - np.float32(SHI))
NZ = 1024
NS = env('NS', 4); NXA = env('NXA', 3); NY = env('NY', 2); NH = 2; NP = 2
TAPS = [0, 1, 2, 3, 5, 6, 7, 8]

def kern(zz, x_hbm, dw_ref, w1_ref, b1_ref, w2t_ref, b2_ref, gam_ref, o_hbm, *scr):
    k = 0
    def take(n):
        nonlocal k
        r = scr[k:k + n]; k += n
        return r
    xf = take(NS); xas = take(NXA); ybs = take(NY); hsc = take(NH); pms = take(NP)
    w1s, w2s, gbs, dsc, dwb_ref = take(5)
    xps = take(NS)
    xbuf, obuf, xsem, osem = take(4)
    i = pl.program_id(0)
    nb = pl.num_programs(0)
    zc = [0]
    def Z(kind):
        if kind in OPQ:
            zc[0] += 1
            return zz[zc[0] % NZ]
        return 0

    NCH = TH // CH
    slot = i % 2
    def x_copy(step, sl, c):
        if c < NCH:
            return pltpu.make_async_copy(x_hbm.at[pl.ds(step * TH + c * CH, CH)], xbuf.at[sl, pl.ds(1 + c * CH, CH)], xsem.at[sl * (NCH + 2) + c])
        if c == NCH:
            return pltpu.make_async_copy(x_hbm.at[pl.ds(jnp.maximum(step * TH - 1, 0), 1)], xbuf.at[sl, pl.ds(0, 1)], xsem.at[sl * (NCH + 2) + c])
        return pltpu.make_async_copy(x_hbm.at[pl.ds(jnp.minimum(step * TH + TH, H - 1), 1)], xbuf.at[sl, pl.ds(TH + 1, 1)], xsem.at[sl * (NCH + 2) + c])
    def o_copy(step, sl, c):
        return pltpu.make_async_copy(obuf.at[sl, pl.ds(c * CH, CH)], o_hbm.at[pl.ds(step * TH + c * CH, CH)], osem.at[sl * NCH + c])
    order = [NCH] + list(range(NCH)) + [NCH + 1]
    @pl.when(i == 0)
    def _():
        for c in order: x_copy(0, 0, c).start()
    @pl.when(i >= 2)
    def _():
        for c in range(NCH): o_copy(i - 2, slot, c).wait()
    @pl.when(i + 1 < nb)
    def _():
        for c in order: x_copy(i + 1, 1 - slot, c).start()
    @pl.when(i == 0)
    def _():
        def col(rowv):
            r = jnp.concatenate([rowv, jnp.zeros((1, 128 - C), f32)], axis=1)
            return jnp.broadcast_to(r, (128, 128)).T[:C]
        dwv = dw_ref[...].astype(f32)
        for ii in range(3):
            for jj in range(3):
                dwb_ref[0, ii * 3 + jj] = col(dwv[ii, jj:jj + 1, :])
        gam = gam_ref[...].astype(f32).reshape(1, C)
        b2v = b2_ref[...].astype(f32).reshape(1, C)
        gbs[0] = col(gam * b2v)
        gsc_ = col(gam * (0.5 / S))
        for kk in range(3):
            w2s[0, kk] = pltpu.bitcast((w2t_ref[:, kk * 128:(kk + 1) * 128].astype(f32) * gsc_).astype(bf16), u32)
        w1f = w1_ref[...].astype(f32)
        b1v = b1_ref[...].astype(f32).reshape(1, E)
        cs = -jnp.sum(w1f, axis=0, keepdims=True)
        s8 = lax.broadcasted_iota(jnp.int32, (8, E), 0)
        ex = jnp.where(s8 < 2, b1v, jnp.where(s8 == 2, cs if KPAD else 0.0, 0.0))
        w1p = jnp.concatenate([w1f, ex, jnp.zeros((24, E), f32)], axis=0)
        w1s[0] = pltpu.bitcast(w1p.T.astype(bf16), u32)
        sub = lax.broadcasted_iota(jnp.int32, (32, W), 0)
        padc = jnp.where(sub == 0, SHI, jnp.where(sub == 1, SLO, 0.0)).astype(f32)
        for xa in xas: xa[0, C:, :] = padc
        r16 = lax.broadcasted_iota(jnp.int32, (16, 128), 0); l16 = lax.broadcasted_iota(jnp.int32, (16, 128), 1)
        for q in range(GM):
            d = jnp.zeros((16, 128), f32)
            for ti, tap in enumerate(TAPS):
                d = jnp.where(l16 == r16 + 16 * ti, dwb_ref[0, tap, 16 * q:16 * q + 16, :], d)
            dsc[0, q] = pltpu.bitcast(d.astype(bf16), u32)

    xin = xbuf.at[slot]
    o_ref = obuf.at[slot]

    lane = lax.broadcasted_iota(jnp.int32, (8, 128), 1)
    sub8 = lax.broadcasted_iota(jnp.int32, (8, 128), 0)
    m_first = lane == 0
    m_last = lane == 127

    def unpack(v):
        s = (v + 1) % NS
        ok = None
        if v < 0:
            if not NOWAIT: x_copy(i, slot, NCH).wait()
            src = xin.at[0]; ok = i > 0
        elif v >= TH:
            if not NOWAIT: x_copy(i, slot, NCH + 1).wait()
            src = xin.at[TH + 1]; ok = i < nb - 1
        else:
            if v % CH == 0 and not NOWAIT: x_copy(i, slot, v // CH).wait()
            src = xin.at[1 + v]
        x = src[...].astype(f32)
        if ok is not None: x = jnp.where(ok, x, 0.0)
        xf[s][0] = x
        if GM:
            pk = pltpu.bitcast(src[0:16 * GM, :], u32)
            if ok is not None: pk = jnp.where(ok, pk, jnp.zeros((), u32))
            xps[s][0, 0] = pk
            z0 = jnp.zeros((8, 128), u32)
            for q in range(GM):
                sl = slice(8 * q, 8 * q + 8)
                pm = [pltpu.roll(pk[sl, t * 128:(t + 1) * 128], 1, 1) for t in range(4)]
                pp = [pltpu.roll(pk[sl, t * 128:(t + 1) * 128], 127, 1) for t in range(4)]
                for t in range(4):
                    ln = slice(t * 128, (t + 1) * 128)
                    xps[s][0, 1, sl, ln] = jnp.where(m_first, pm[t - 1] if t > 0 else z0, pm[t])
                    xps[s][0, 2, sl, ln] = jnp.where(m_last, pp[t + 1] if t < 3 else z0, pp[t])
    XF = lambda v: xf[(v + 1) % NS]
    XP = lambda v: xps[(v + 1) % NS]

    AS = {}
    def acc(v, t, y, sl, ln):
        st = AS[v]
        if YV: st.setdefault('y', {})[(sl.start, ln.start)] = y
        else: ybs[v % NY][0, sl, ln] = y
        q = t + 4 * ((sl.start // 8) % SACC)
        st['s1'][q] = y if st['s1'][q] is None else st['s1'][q] + y
        st['s2'][q] = y * y if st['s2'][q] is None else st['s2'][q] + y * y
    def a_begin(v):
        AS[v] = dict(s1=[None] * (4 * SACC), s2=[None] * (4 * SACC), za=[Z('x') for _ in range(3)], zd=Z('d'), zp=[Z('q') for _ in range(3)])
    def a_mxu(v, q):
        st = AS[v]
        parts = []
        for tap in TAPS:
            ii, j = divmod(tap, 3)
            parts.append(pltpu.bitcast(XP(v - 1 + ii)[st['zp'][ii], (1, 0, 2)[j], 8 * q:8 * q + 8, :], bf16))
        rhs = jnp.concatenate(parts, axis=0)
        y = jnp.dot(pltpu.bitcast(dsc[st['zd'], q], bf16), rhs, preferred_element_type=f32)
        for hh in range(2):
            sl = slice(16 * q + 8 * hh, 16 * q + 8 * hh + 8)
            w4 = dwb_ref[st['zd'], 4, sl, :]
            for t in range(4):
                ln = slice(t * 128, (t + 1) * 128)
                acc(v, t, y[8 * hh:8 * hh + 8, ln] + XF(v)[st['za'][1], sl, ln] * w4, sl, ln)
    def a_valu(v, g):
        st = AS[v]; za = st['za']
        sl = slice(g * 8, (g + 1) * 8)
        wts = [dwb_ref[st['zd'], kk, sl, :] for kk in range(9)]
        ym = []; y0 = []; yp = []
        for t in range(4):
            ln = slice(t * 128, (t + 1) * 128)
            a = XF(v - 1)[za[0], sl, ln]; b = XF(v)[za[1], sl, ln]; c = XF(v + 1)[za[2], sl, ln]
            ym.append(pltpu.roll(a * wts[0] + b * wts[3] + c * wts[6], 1, 1))
            y0.append(a * wts[1] + b * wts[4] + c * wts[7])
            yp.append(pltpu.roll(a * wts[2] + b * wts[5] + c * wts[8], 127, 1))
        for t in range(4):
            ln = slice(t * 128, (t + 1) * 128)
            l = jnp.where(m_first, ym[t - 1] if t > 0 else 0.0, ym[t])
            rr = jnp.where(m_last, yp[t + 1] if t < 3 else 0.0, yp[t])
            acc(v, t, (y0[t] + l + rr) if YA == 0 else (y0[t] + (l + rr)), sl, ln)
    def a_ln(v):
        st = AS.pop(v); s1 = st['s1']; s2 = st['s2']
        for q in range(1, SACC):
            for t in range(4):
                s1[t] = s1[t] + s1[4 * q + t]; s2[t] = s2[t] + s2[4 * q + t]
        yb = ybs[v % NY]; xa = xas[v % NXA]
        zy = Z('y')
        pc = jnp.where(sub8 == 0, SHI, jnp.where(sub8 == 1, SLO, 0.0)).astype(f32)
        def stats(a1, a2):
            m = a1 * (1.0 / C)
            vv = a2 * (1.0 / C) - m * m
            rs = lax.rsqrt(jnp.maximum(vv, 0.0) + 1e-5) * S
            return m, rs
        if STAT == 0:
            ms = []; rss = []
            for t in range(4):
                m, rs = stats(jnp.sum(s1[t], axis=0, keepdims=True), jnp.sum(s2[t], axis=0, keepdims=True))
                ms.append(jnp.broadcast_to(m, (8, 128))); rss.append(jnp.broadcast_to(rs, (8, 128)))
        else:
            def merge(vs):
                lo = sub8 < 4
                ev = (sub8 % 2) == 0
                def fold4(a): return a + pltpu.roll(a, 4, 0)
                def comb(a, b, sh, msk):
                    u = jnp.where(msk, a, b); w = jnp.where(msk, b, a)
                    return u + pltpu.roll(w, sh, 0) if False else u + rollx(w, sh, msk)
                def rollx(w, sh, msk):
                    return jnp.where(msk, pltpu.roll(w, 8 - sh, 0), pltpu.roll(w, sh, 0)) if sh != 4 else pltpu.roll(w, 4, 0)
                return None
            r1 = [jnp.broadcast_to(jnp.sum(s1[t], axis=0, keepdims=True), (8, 128)) for t in range(4)]
            r2 = [jnp.broadcast_to(jnp.sum(s2[t], axis=0, keepdims=True), (8, 128)) for t in range(4)]
            g1 = jnp.where(sub8 < 2, r1[0], jnp.where(sub8 < 4, r1[1], jnp.where(sub8 < 6, r1[2], r1[3])))
            g2 = jnp.where(sub8 < 2, r2[0], jnp.where(sub8 < 4, r2[1], jnp.where(sub8 < 6, r2[2], r2[3])))
            m, rs = stats(g1, g2)
            ms = [jnp.broadcast_to(m[2 * t:2 * t + 1, :], (8, 128)) for t in range(4)]
            rss = [jnp.broadcast_to(rs[2 * t:2 * t + 1, :], (8, 128)) for t in range(4)]
        cols = []
        for t in range(4):
            ln = slice(t * 128, (t + 1) * 128)
            rsb = rss[t]; mb = ms[t]
            for _ in range(NHOP): rsb = pltpu.roll(rsb, Z('r'), 1)
            parts = []
            for g in range(C // 8):
                sl = slice(g * 8, (g + 1) * 8)
                yy = st['y'][(sl.start, ln.start)] if YV else yb[zy, sl, ln]
                val = yy * rsb if KPAD else (yy - mb) * rsb
                if AV: parts.append(val)
                else: xa[0, sl, ln] = val
            pv = jnp.where(sub8 == 2, mb * rsb, pc) if KPAD else pc
            if AV:
                cols.append(jnp.concatenate(parts + [pv, jnp.zeros((24, 128), f32)], axis=0))
            elif KPAD:
                xa[0, 96:104, ln] = pv
        if AV: XAV[v] = jnp.concatenate(cols, axis=1)
    XAV = {}

    def mm1(v):
        w1 = pltpu.bitcast(w1s[Z('w')], bf16)
        hsc[v % NH][0] = jnp.dot(w1, XAV.pop(v) if AV else xas[v % NXA][Z('a')], preferred_element_type=f32)
    def mm2(v, hook):
        zw = Z('w')
        h = hsc[v % NH][Z('h')]
        tt = jnp.tanh(h * (h * h + KK))
        g = h + h * tt if GEL == 0 else h * (1.0 + tt)
        gb = jnp.concatenate([gbs[zw]] * 4, axis=1)
        pm = pms[v % NP]
        npm = 3 if PMEM == 1 else 2
        last = None
        for kk in range(3):
            p = jnp.dot(pltpu.bitcast(w2s[zw, kk], bf16), g[kk * 128:(kk + 1) * 128], preferred_element_type=f32)
            if kk < npm: pm[0, kk] = p
            else: last = p
            hook(kk + 1)
        zp = Z('p')
        a = pm[zp, 0] + pm[zp, 1]
        a = a + (pm[zp, 2] if PMEM == 1 else last)
        xr = XF(v)[Z('o')]
        if OUTA == 0: ov = a + (xr + gb)
        elif OUTA == 1: ov = (a + xr) + gb
        elif OUTA == 2: ov = (pm[zp, 0] + xr) + (pm[zp, 1] + gb) + last
        else: ov = (a + gb) + xr
        o_ref[v] = ov.astype(bf16)

    def stageA_parts(v):
        unpack(v + 1); a_begin(v)
        return [functools.partial(a_mxu, v, q) for q in range(GM)], [functools.partial(a_valu, v, g) for g in range(2 * GM, C // 8)]
    if NOWAIT:
        for c in order: x_copy(i, slot, c).wait()
    unpack(-1); unpack(0)
    AL = env('AL', 1)
    for v in range(AL):
        mx, va = stageA_parts(v)
        for o in mx + va: o()
        a_ln(v)
    nxt = AL
    if AL == 1 or True:
        pass
    mm1(0)
    D = [int(c) for c in DIST]
    for r in range(TH):
        m = r + AL
        mx, va = ([], [])
        if m < TH: mx, va = stageA_parts(m)
        q = [0]
        def hook(hh):
            for _ in range(D[hh]):
                if q[0] < len(mx): mx[q[0]](); q[0] += 1
        if r % CH == LAGC % CH and r >= CH: o_copy(i, slot, r // CH - 1).start()
        if AL == 1 or not GM:
            for o in mx + va: o()
            q[0] = len(mx)
            if m < TH: a_ln(m)
            if r + 1 < TH: mm1(r + 1)
            mm2(r, lambda hh: None)
        else:
            if r + 1 < TH: mm1(r + 1)
            hook(0)
            mm2(r, hook)
            while q[0] < len(mx): mx[q[0]](); q[0] += 1
            for o in va: o()
            if m < TH: a_ln(m)

    o_copy(i, slot, NCH - 1).start()
    @pl.when(i == nb - 1)
    def _():
        for c in range(NCH): o_copy(i - 1, 1 - slot, c).wait()
        for c in range(NCH): o_copy(i, slot, c).wait()

@jax.jit
def pallas_standalone__modern_conv_block_convnext__vision_kernel(x, dw, w1, b1, w2, b2, gamma):
    xt = jnp.transpose(x[0], (0, 2, 1))
    w2t = w2.T
    nb = H // TH
    zz = jnp.zeros((NZ,), jnp.int32)
    full = lambda a: pl.BlockSpec(a.shape, lambda i, z: (0,) * a.ndim)
    scr = [pltpu.VMEM((1, C, W), f32)] * NS + [pltpu.VMEM((1, 128, W), f32)] * NXA + [pltpu.VMEM((1, C, W), f32)] * NY
    scr += [pltpu.VMEM((1, E, W), f32)] * NH + [pltpu.VMEM((1, 3, C, W), f32)] * NP
    scr += [pltpu.VMEM((1, E // 2, 128), u32), pltpu.VMEM((1, 3, C // 2, 128), u32), pltpu.VMEM((1, C, 128), f32), pltpu.VMEM((1, max(GM, 1), 8, 128), u32), pltpu.VMEM((1, 9, C, 128), f32)]
    scr += [pltpu.VMEM((1, 3, 8 * max(GM, 1), W), u32)] * NS
    NCH = TH // CH
    scr += [pltpu.VMEM((2, TH + 2, C, W), bf16), pltpu.VMEM((2, TH, C, W), bf16), pltpu.SemaphoreType.DMA((2 * (NCH + 2),)), pltpu.SemaphoreType.DMA((2 * NCH,))]
    out = pl.pallas_call(
        kern,
        grid_spec=pltpu.PrefetchScalarGridSpec(
            num_scalar_prefetch=1, grid=(nb,),
            in_specs=[pl.BlockSpec(memory_space=pl.ANY), full(dw), full(w1), full(b1), full(w2t), full(b2), full(gamma)],
            out_specs=pl.BlockSpec(memory_space=pl.ANY),
            scratch_shapes=scr),
        out_shape=jax.ShapeDtypeStruct((H, C, W), bf16),
        compiler_params=pltpu.CompilerParams(dimension_semantics=("arbitrary",), vmem_limit_bytes=110 * 1024 * 1024, flags=FLAGS),
    )(zz, xt, dw, w1, b1, w2t, b2, gamma)
    return jnp.transpose(out, (0, 2, 1))[None]
```

```python
import numpy as np
import jax
import jax.numpy as jnp
from jax import lax
from jax.experimental import pallas as pl
from jax.experimental.pallas import tpu as pltpu


H = 512; W = 512; C = 96; E = 384
F0 = 16
TB = 62
NBIG = (H - F0) // TB
assert F0 + NBIG * TB == H
def chunks(s):
    c = [int(x) for x in s.split(',')]
    return c
OC = chunks('31,15,8,4,4')
OC0 = chunks('16')
assert sum(OC) == TB and sum(OC0) == F0
XCH = 1
XC0 = chunks('4,13')
assert sum(XC0) == F0 + 1
NODX = 0; NODO = 0
NS = 6; NY = 2; NH = 2; NP = 2
NZ = 1024
f32 = jnp.float32; bf16 = jnp.bfloat16; u32 = jnp.uint32
C1 = float(np.sqrt(2.0 / np.pi)); C2 = 0.044715
S = float((C1 * C2) ** (1.0 / 3.0)); KK = C1 / S
SHI = float(np.float32(S).astype(jnp.bfloat16).astype(np.float32)); SLO = float(np.float32(S) - np.float32(SHI))
NOC = max(len(OC), len(OC0))
NXS = XCH + 1


YL = 3; GEL = 1; OUTA = 0; CO = 3; OPQ = 'hopyw'; SZ = 1; LATE = 0; MANW = 1; SKIPW = 0
def kern(zz, x_hbm, dw_ref, w1_ref, b1_ref, w2t_ref, b2_ref, gam_ref, o_hbm, *scr):
    if MANW:
        wsrc = (dw_ref, w1_ref, b1_ref, w2t_ref, b2_ref, gam_ref)
        wdst = scr[-7:-1]; wsem = scr[-1]; scr = scr[:-7]
        dw_ref, w1_ref, b1_ref, w2t_ref, b2_ref, gam_ref = wdst
        w_copies = lambda: [pltpu.make_async_copy(a, b, wsem.at[k]) for k, (a, b) in enumerate(zip(wsrc, wdst))]
    xf = scr[:NS]; ybs = scr[NS:NS + NY]; hsc = scr[NS + NY:NS + NY + NH]; pms = scr[NS + NY + NH:NS + NY + NH + NP]
    w1s, w2s, gbs, dwb_ref, xbuf, obuf, xsem, osem = scr[NS + NY + NH + NP:]
    i = pl.program_id(0)
    nb = pl.num_programs(0)
    zc = [0]

    def Z(kind='z'):
        if kind != 'z' and kind not in OPQ: return 0
        zc[0] += 1
        return zz[zc[0] % NZ]

    slot = i % 2
    row0 = lambda step: F0 + (step - 1) * TB
    xsz = [(TB + 1 + k) // XCH for k in range(XCH)]
    xoff = [sum(xsz[:k]) for k in range(XCH)]

    def x_copies(step, sl):
        r0 = row0(step)
        cs = [pltpu.make_async_copy(x_hbm.at[pl.ds(r0 - 1 + xoff[k], xsz[k])], xbuf.at[sl, pl.ds(xoff[k], xsz[k])], xsem.at[sl * NXS + k]) for k in range(XCH)]
        cs.append(pltpu.make_async_copy(x_hbm.at[pl.ds(jnp.minimum(r0 + TB, H - 1), 1)], xbuf.at[sl, pl.ds(TB + 1, 1)], xsem.at[sl * NXS + XCH]))
        return cs

    def x0_copies():
        return [pltpu.make_async_copy(x_hbm.at[pl.ds(sum(XC0[:k]), XC0[k])], xbuf.at[0, pl.ds(1 + sum(XC0[:k]), XC0[k])], xsem.at[2 * NXS + k]) for k in range(len(XC0))]

    def o_copy(r0, sl, oc, c):
        off = sum(oc[:c])
        return pltpu.make_async_copy(obuf.at[sl, pl.ds(off, oc[c])], o_hbm.at[pl.ds(r0 + off, oc[c])], osem.at[sl * NOC + c])

    def o_wait(step_pred_small, step, sl):
        pass

    @pl.when(i == 0)
    def _():
        if not NODX:
            cs = x0_copies()
            cs[0].start()
            if MANW:
                for c in w_copies(): c.start()
            if not LATE:
                for c in cs[1:]: c.start()

    if not NODO:
        @pl.when(i == 2)
        def _():
            for c in range(len(OC0)): o_copy(0, 0, OC0, c).wait()

        @pl.when(i > 2)
        def _():
            for c in range(len(OC)): o_copy(row0(i - 2), slot, OC, c).wait()

    if SKIPW:
        @pl.when(i == 2)
        def _():
            for c in x_copies(1, 1): c.wait()
    if not NODX:
        @pl.when((i + 1 < nb) & (i > 0) if LATE else (i + 1 < nb))
        def _():
            for c in x_copies(i + 1, 1 - slot): c.start()

    @pl.when(i == 0)
    def _():
        if MANW:
            for c in w_copies(): c.wait()
        def col(rowv):
            r = jnp.concatenate([rowv, jnp.zeros((1, 128 - C), f32)], axis=1)
            return jnp.broadcast_to(r, (128, 128)).T[:C]
        dwv = dw_ref[...].astype(f32)
        for ii in range(3):
            for jj in range(3):
                dwb_ref[0, ii * 3 + jj] = col(dwv[ii, jj:jj + 1, :])
        gam = gam_ref[...].astype(f32).reshape(1, C)
        b2v = b2_ref[...].astype(f32).reshape(1, C)
        gbs[0] = col(gam * b2v)
        gsc = col(gam * (0.5 / S))
        for kk in range(3):
            w2s[0, kk] = pltpu.bitcast((w2t_ref[:, kk * 128:(kk + 1) * 128].astype(f32) * gsc).astype(bf16), u32)
        w1f = w1_ref[...].astype(f32)
        b1v = b1_ref[...].astype(f32).reshape(1, E)
        cs = -jnp.sum(w1f, axis=0, keepdims=True)
        s8 = lax.broadcasted_iota(jnp.int32, (8, E), 0)
        ex = jnp.where(s8 < 2, b1v, jnp.where(s8 == 2, cs, 0.0))
        w1p = jnp.concatenate([w1f, ex, jnp.zeros((24, E), f32)], axis=0)
        w1s[0] = pltpu.bitcast(w1p.T.astype(bf16), u32)

    lane = lax.broadcasted_iota(jnp.int32, (8, 128), 1)
    sub8 = lax.broadcasted_iota(jnp.int32, (8, 128), 0)
    m_first = lane == 0
    m_last = lane == 127
    XF = lambda v: xf[(v + 1) % NS]

    def body(T, xin, o_ref, first, r0, sl, oc):
        def unpack(v):
            if v < 0 and first:
                XF(v)[0] = jnp.zeros((C, W), f32)
                return
            if first and v in xw and not NODX:
                x0_copies()[xw[v]].wait()
                if LATE == 1 and xw[v] == 0:
                    for c in x0_copies()[1:] + x_copies(1, 1): c.start()
                if LATE == 2:
                    if xw[v] + 1 < len(XC0): x0_copies()[xw[v] + 1].start()
                    else:
                        for c in x_copies(1, 1): c.start()
            x = xin[1 + v].astype(f32)
            if v >= T and not first: x = jnp.where(i < nb - 1, x, 0.0)
            XF(v)[0] = x

        XAV = {}
        xw = {sum(XC0[:k]): k for k in range(len(XC0))}

        def stage_a(v):
            unpack(v + 1)
            s1 = [None] * 4; s2 = [None] * 4
            yb = ybs[v % NY]
            for g in range(C // 8):
                sl = slice(g * 8, (g + 1) * 8)
                wts = [dwb_ref[0, kk, sl, :] for kk in range(9)]
                ym = []; y0 = []; yp = []
                for t in range(4):
                    ln = slice(t * 128, (t + 1) * 128)
                    a = XF(v - 1)[0, sl, ln]; b = XF(v)[0, sl, ln]; c = XF(v + 1)[0, sl, ln]
                    def f0():
                        if YL == 0: y0.append(a * wts[1] + b * wts[4] + c * wts[7])
                        else: yb[0, sl, ln] = a * wts[1] + b * wts[4] + c * wts[7]
                    def fm(): ym.append(pltpu.roll(a * wts[0] + b * wts[3] + c * wts[6], 1, 1))
                    def fp(): yp.append(pltpu.roll(a * wts[2] + b * wts[5] + c * wts[8], 127, 1))
                    for ch in ('m0p', '0mp', 'mp0', 'pm0', 'p0m')[CO]: {'m': fm, '0': f0, 'p': fp}[ch]()
                for t in range(4):
                    ln = slice(t * 128, (t + 1) * 128)
                    l = jnp.where(m_first, ym[t - 1] if t > 0 else 0.0, ym[t])
                    r = jnp.where(m_last, yp[t + 1] if t < 3 else 0.0, yp[t])
                    y = (y0[t] if YL == 0 else yb[0, sl, ln]) + (l + r)
                    yb[0, sl, ln] = y
                    s1[t] = y if s1[t] is None else s1[t] + y
                    s2[t] = y * y if s2[t] is None else s2[t] + y * y
            zy = Z('y')
            pc = jnp.where(sub8 == 0, SHI, jnp.where(sub8 == 1, SLO, 0.0)).astype(f32)
            ms = []; rss = []
            for t in range(4):
                m = jnp.sum(s1[t], axis=0, keepdims=True) * (1.0 / C)
                var = jnp.sum(s2[t], axis=0, keepdims=True) * (1.0 / C) - m * m
                rs = lax.rsqrt(jnp.maximum(var, 0.0) + 1e-5) * S
                ms.append(jnp.broadcast_to(m, (8, 128))); rss.append(jnp.broadcast_to(rs, (8, 128)))
            cols = []
            for t in range(4):
                ln = slice(t * 128, (t + 1) * 128)
                parts = [yb[zy, g * 8:(g + 1) * 8, ln] * rss[t] for g in range(C // 8)]
                pv = jnp.where(sub8 == 2, ms[t] * rss[t], pc)
                cols.append(jnp.concatenate(parts + [pv, jnp.zeros((24, 128), f32)], axis=0))
            XAV[v] = jnp.concatenate(cols, axis=1)

        def mm1(v):
            w1 = pltpu.bitcast(w1s[Z('w')], bf16)
            hsc[v % NH][0] = jnp.dot(w1, XAV.pop(v), preferred_element_type=f32)

        def mm2(v):
            zw = Z('w')
            zh = Z('h')
            gb = jnp.concatenate([gbs[0]] * 4, axis=1)
            pm = pms[v % NP]
            for kk in range(3):
                h = hsc[v % NH][zh if SZ else Z('h'), kk * 128:(kk + 1) * 128]
                tt = jnp.tanh(h * (h * h + KK))
                g = h + h * tt if GEL == 0 else h * (1.0 + tt)
                p = jnp.dot(pltpu.bitcast(w2s[zw, kk], bf16), g, preferred_element_type=f32)
                if kk < 2: pm[0, kk] = p
            zp = Z('p')
            a = pm[zp, 0] + pm[zp, 1] + p
            xr = XF(v)[Z('o')]
            if OUTA == 0: ov = a + (xr + gb)
            elif OUTA == 1: ov = (a + xr) + gb
            elif OUTA == 2: ov = (pm[zp, 0] + xr) + (pm[zp, 1] + gb) + p
            else: ov = (a + gb) + xr
            o_ref[v] = ov.astype(bf16)

        starts = {}
        off = 0
        for c in range(len(oc) - 1):
            off += oc[c]; starts[off] = c
        unpack(-1); unpack(0)
        stage_a(0)
        mm1(0)
        for r in range(T):
            if r in starts and not NODO: o_copy(r0, sl, oc, starts[r]).start()
            if r + 1 < T:
                stage_a(r + 1)
                mm1(r + 1)
            mm2(r)
        if not NODO: o_copy(r0, sl, oc, len(oc) - 1).start()

    @pl.when(i == 0)
    def _():
        body(F0, xbuf.at[0], obuf.at[0], True, 0, 0, OC0)

    @pl.when(i > 0)
    def _():
        if not NODX and not SKIPW:
            for c in x_copies(i, slot): c.wait()
        if SKIPW:
            @pl.when(i > 1)
            def _():
                for c in x_copies(i, slot): c.wait()
        body(TB, xbuf.at[slot], obuf.at[slot], False, row0(i), slot, OC)

    if not NODO:
        @pl.when(i == nb - 1)
        def _():
            for c in range(len(OC)): o_copy(row0(i - 1), 1 - slot, OC, c).wait()
            for c in range(len(OC)): o_copy(row0(i), slot, OC, c).wait()


@jax.jit
def pallas_standalone__modern_conv_block_convnext__vision_kernel(x, dw, w1, b1, w2, b2, gamma):
    xt = jnp.transpose(x[0], (0, 2, 1))
    w2t = w2.T
    nb = NBIG + 1
    zz = jnp.zeros((NZ,), jnp.int32)
    full = lambda a: pl.BlockSpec(a.shape, lambda i, z: (0,) * a.ndim)
    scr = [pltpu.VMEM((1, C, W), f32)] * NS + [pltpu.VMEM((1, C, W), f32)] * NY
    scr += [pltpu.VMEM((1, E, W), f32)] * NH + [pltpu.VMEM((1, 3, C, W), f32)] * NP
    scr += [pltpu.VMEM((1, E // 2, 128), u32), pltpu.VMEM((1, 3, C // 2, 128), u32), pltpu.VMEM((1, C, 128), f32), pltpu.VMEM((1, 9, C, 128), f32)]
    scr += [pltpu.VMEM((2, TB + 2, C, W), bf16), pltpu.VMEM((2, TB, C, W), bf16),
            pltpu.SemaphoreType.DMA((2 * NXS + len(XC0),)), pltpu.SemaphoreType.DMA((2 * NOC,))]
    anys = pl.BlockSpec(memory_space=pl.ANY)
    ws = [dw, w1, b1, w2t, b2, gamma]
    if MANW:
        scr += [pltpu.VMEM(a.shape, a.dtype) for a in ws] + [pltpu.SemaphoreType.DMA((6,))]
    out = pl.pallas_call(
        kern,
        grid_spec=pltpu.PrefetchScalarGridSpec(
            num_scalar_prefetch=1, grid=(nb,),
            in_specs=[anys] + ([anys] * 6 if MANW else [full(a) for a in ws]),
            out_specs=pl.BlockSpec(memory_space=pl.ANY),
            scratch_shapes=scr),
        out_shape=jax.ShapeDtypeStruct((H, C, W), bf16),
        compiler_params=pltpu.CompilerParams(dimension_semantics=("arbitrary",), vmem_limit_bytes=110 * 1024 * 1024),
    )(zz, xt, dw, w1, b1, w2t, b2, gamma)
    return jnp.transpose(out, (0, 2, 1))[None]
```
